```python
import os as _os
_os.environ.setdefault('JAX_PLATFORMS', 'cpu')
import jax
import jax.numpy as jnp

def _softmax(x, axis=-1):
    return jax.nn.softmax(x, axis=axis)

def _gelu(x):
    return jax.nn.gelu(x, approximate=True)

def _silu(x):
    return jax.nn.silu(x)

def _sigmoid(x):
    return jax.nn.sigmoid(x)

def _layernorm(x, axis=-1, eps=1e-05):
    m = jnp.mean(x, axis=axis, keepdims=True)
    v = jnp.var(x, axis=axis, keepdims=True)
    return (x - m) / jnp.sqrt(v + eps)

def _scatter_add(tgt, idx, src, axis=0):
    return tgt.at[idx].add(src)

def _segment_sum(src, seg, n):
    return jax.ops.segment_sum(src, seg, n)

class _Rng:

    def __init__(self, key):
        self._k = key

    def _next(self):
        self._k, sub = jax.random.split(self._k)
        return sub

    def normal(self, shape):
        return jax.random.normal(self._next(), shape, dtype=jnp.bfloat16)

    def randint(self, lo, hi, shape):
        return jax.random.randint(self._next(), shape, lo, hi, dtype=jnp.int32)

    def uniform(self, shape, lo=0.0, hi=1.0):
        return jax.random.uniform(self._next(), shape, jnp.bfloat16, lo, hi)

    def permutation(self, n):
        return jax.random.permutation(self._next(), n)
kernel_name = 'adaLN_cond__sliding_local_dilated__dense_activation_gelu__prompt'

def setup_inputs():
    _rng = _Rng(jax.random.key(int.from_bytes(__import__("os").urandom(4), "little")))
    _w = lambda a: (lambda t: t.astype(jnp.bfloat16) if jnp.issubdtype(t.dtype, jnp.floating) else t)(jnp.asarray(a))

    def _A_setup():
        B, S, D = (1, 2048, 576)
        return {'x': _w((lambda *s: _rng.normal(s) * 0.05)(B, S, D)), 'wqkv': _w((lambda *s: _rng.normal(s) * 0.05)(D, 3 * D)), 'wo': _w((lambda *s: _rng.normal(s) * 0.05)(D, D))}
    _A_in = _A_setup()

    def _B_setup():
        B, S, D, F = (1, 2048, 576, 4608)
        return {'x': _w((lambda *s: _rng.normal(s) * 0.05)(B, S, D)), 'w1': _w((lambda *s: _rng.normal(s) * 0.8)(D, F) * D ** (-0.5)), 'b1': _w((lambda *s: _rng.normal(s) * 0.8)(F) * 0.01), 'w2': _w((lambda *s: _rng.normal(s) * 0.8)(F, D) * F ** (-0.5)), 'b2': _w((lambda *s: _rng.normal(s) * 0.8)(D) * 0.01)}
    _B_in = _B_setup()
    return {'A_x': _A_in['x'], 'A_wqkv': _A_in['wqkv'], 'A_wo': _A_in['wo'], 'B_x': _B_in['x'], 'B_w1': _B_in['w1'], 'B_b1': _B_in['b1'], 'B_w2': _B_in['w2'], 'B_b2': _B_in['b2'], 'c': _w((lambda *s: _rng.normal(s) * 0.05)(1, 576) * 8.0), 'w_mod': _w((lambda *s: _rng.normal(s) * 0.05)(576, 6 * 576) * 576 ** (-0.5) * 8.0)}

def reference(A_x, A_wqkv, A_wo, B_x, B_w1, B_b1, B_w2, B_b2, c, w_mod):

    def _A_ref(x, wqkv, wo):
        B, S, D = x.shape
        H = 32
        Dh = D // H
        W, dil = (8, 2)
        qkv = (lambda x, *d: x.transpose(*d))((x @ wqkv).reshape(B, S, 3, H, Dh), 2, 0, 3, 1, 4)
        q, k, v = (qkv[0], qkv[1], qkv[2])
        scale = Dh ** (-0.5)
        pos = jnp.arange(S)
        off = jnp.arange(W) * dil
        idx = pos[:, None] - off[None, :]
        mask = idx >= 0
        idx_c = jnp.where(mask, idx, 0).reshape(-1)
        kg = k[:, :, idx_c, :].reshape(B, H, S, W, Dh)
        vg = v[:, :, idx_c, :].reshape(B, H, S, W, Dh)
        logits = jnp.einsum('bhsd,bhswd->bhsw', q, kg) * scale
        logits = jnp.where(mask[None, None, :, :], logits, -1000000000.0)
        attn = _softmax(logits, axis=-1)
        o = jnp.einsum('bhsw,bhswd->bhsd', attn, vg)
        return (lambda x, *d: x.transpose(*d))(o, 0, 2, 1, 3).reshape(B, S, D) @ wo

    def _B_ref(x, w1, b1, w2, b2):
        h = jnp.einsum('bsd,df->bsf', x, w1) + b1
        h = _gelu(h)
        return jnp.einsum('bsf,fd->bsd', h, w2) + b2
    x = A_x
    mod = (_silu(c) @ w_mod).reshape(c.shape[0], 6, 1, -1)
    sa, ca, ga, sb, cb, gb = (mod[:, 0].copy(), mod[:, 1].copy(), mod[:, 2].copy(), mod[:, 3].copy(), mod[:, 4].copy(), mod[:, 5].copy())
    h = _layernorm(x, axis=-1) * (1 + ca) + sa
    x = x + ga * _A_ref(h, A_wqkv, A_wo)
    h = _layernorm(x, axis=-1) * (1 + cb) + sb
    x = x + gb * _B_ref(h, B_w1, B_b1, B_w2, B_b2)
    return x
```

```python
import functools
import math

import jax
import jax.numpy as jnp
from jax import lax
import jax.experimental.pallas as pl
import jax.experimental.pallas.tpu as pltpu

F32, BF16, U32 = jnp.float32, jnp.bfloat16, jnp.uint32
P = functools.partial
_memo = functools.lru_cache(maxsize=None)

S, D, F = 2048, 576, 4608
DH, W, DIL = 18, 8, 2
EPS = 1e-5
L = 128
NT = S // L
G = 4
R = D // G
NB = NT // 4
NC = F // (4 * L)
HW = W // 2
GS = HW * DIL

X0, X1 = 4, 8
T_WAVE3, T_WAVE4 = 4.25, 12.0
T_MOD, T_LN, T_PREP, T_MLP = 5.0, 0.5, 12.5, 16.0
ATT_STEP = (0.55, 0.85, 0.4)
ATT_LAG = (2, 4, 5, 7)
PROJ_FROM, PROJ_EARLY = 8, 9
SPANS = (2, 3, 4)
LEAD = 810
DU = 6
RP = D // 6

_SA = (((0, 1), (3, 1)), ((2, 1), (3, 1)), ((0, 1),), ((3, 1),),
       ((0, 1), (1, 1)), ((2, 1), (0, -1)), ((1, 1), (3, -1)))
_SB = (((0, 1), (3, 1)), ((0, 1),), ((1, 1), (3, -1)), ((2, 1), (0, -1)),
       ((3, 1),), ((0, 1), (1, 1)), ((2, 1), (3, 1)))
_REM = {2: (((0, 1),), 1), 3: (((1, 1),), 0), 5: (((1, 1), (0, -1)), 1), 6: (((0, 1), (1, -1)), 0)}
_OUTER = (1, 3, 2, 4, 0, 6, 5)
_UP = [(o, i) for o in _OUTER for i in (0, 1, 3, 6, 2, 4, 5, 7, 9, 8) if i < 7 or o in _REM]
_DOWN = [(o, i) for o in _OUTER for i in (0, 1, 3, 6, 2, 4, 5)]
_DONE = {qo: 7 * max(map(_OUTER.index, need)) + 6
         for qo, need in enumerate(((0, 3, 4, 6), (2, 4), (1, 3), (0, 1, 2, 5)))}

_C = math.sqrt(2.0 / math.pi)
GA = (0.044715 * _C) ** (1.0 / 3.0)


def _comb(terms, get):
    r = None
    for i, s in terms:
        r = get(i) if r is None else (r + get(i) if s > 0 else r - get(i))
    return r


def _result(q, m):
    if q == 0:
        return ((m(0) + m(3)) + m(6)) - m(4)
    if q == 3:
        return (m(0) - m(1)) + (m(2) + m(5))
    return m(2) + m(4) if q == 1 else m(1) + m(3)


def _rc(qo, qi):
    return 2 * (qo // 2) + qi // 2, 2 * (qo % 2) + qi % 2


def _outer(tab, block):
    block = _memo(block)
    return _memo(lambda o, qi: _comb(tab[o], lambda qo: block(*_rc(qo, qi))))


def _tree(op, vals):
    vals = list(vals)
    while len(vals) > 1:
        vals = [op(a, b) for a, b in zip(vals[::2], vals[1::2])] + vals[len(vals) & ~1:]
    return vals[0]


def _vregs(v):
    return [v[k:k + 8] for k in range(0, v.shape[0], 8)]


def _cols(row):
    return jnp.broadcast_to(row, (L, row.shape[1])).astype(BF16).T.astype(F32)


def _merge(*streams):
    out = [((j + 0.5) / len(st), k, f) for k, st in enumerate(streams) for j, f in enumerate(st)]
    return [e[2] for e in sorted(out, key=lambda e: e[:2])]


_X_CUTS = (0, (X0 - 1) * L, X0 * L, X1 * L, S)
_QKV_CUTS = (0, 5 * L, 9 * L, 3 * D)
_MOD_CUTS = (0, 5 * L, 9 * L, 23 * L, 6 * D)


def _kernel(x_hbm, wqkv_hbm, wo_hbm, w1_hbm, b1_hbm, w2t_hbm, b2_hbm, c_hbm, wm_hbm, out_hbm,
            x_v, wqkv_v, wm_v, wo_v, w1_v, b1_v, w2t_v, b2_v, c_v,
            wt32, wo32, wqkv_s, wo_s, h1_s, o_s, hc_s, hr_s, w1c_s, w1r_s, w2c_s, out_v,
            sems, out_sem):
    srcs = [(c_hbm, c_v), (wo_hbm, wo_v), (w1_hbm, w1_v), (w2t_hbm, w2t_v), (b1_hbm, b1_v),
            (b2_hbm, b2_v)]
    for hbm, bufs, cuts in ((x_hbm, x_v, _X_CUTS), (wqkv_hbm, wqkv_v, _QKV_CUTS),
                            (wm_hbm, wm_v, _MOD_CUTS)):
        srcs += [(hbm.at[:, pl.ds(a, b - a)], buf) for buf, a, b in zip(bufs, cuts, cuts[1:])]
    (d_c, d_wo, d_w1, d_w2, d_b1, d_b2, d_x0, d_x1, d_x2, d_x3, d_wq, d_wk, d_wv,
     d_m0, d_m1, d_m2, d_m3) = [
        pltpu.make_async_copy(src, dst, sems.at[k]) for k, (src, dst) in enumerate(srcs)]
    waves = ([d_wk, d_x1], [d_wv, d_x2], [d_x3, d_wo, d_m2], [d_w1, d_w2, d_m3, d_b1, d_b2])

    def start(ds):
        for d in ds:
            d.start()

    def wait(ds):
        for d in ds:
            d.wait()

    def load(bufs, cuts, rows, tile):
        k = max(k for k, a in enumerate(cuts) if a <= tile * L)
        return bufs[k][rows, pl.ds(tile * L - cuts[k], min(L, cuts[-1] - tile * L))]

    def column(row):
        return _cols(jnp.concatenate([row, jnp.zeros((1, 5 * L - D), F32)], axis=1))[:D]

    start([d_c, d_m0, d_m1, d_wq, d_x0])
    d_c.wait()
    c = c_v[...].astype(F32)
    silu_c = column(c * jax.nn.sigmoid(c))

    never = jnp.abs(silu_c[:8]) < 0.0
    pending, issued = [], []

    def token(*vals):
        return _tree(jnp.bitwise_or, [pltpu.bitcast(v, U32) for v in vals])

    def anchor(*vals):
        pending.append(token(*[r for v in vals for r in _vregs(v)]))

    def tied(u):
        if pending:
            rows = _vregs(u)
            for k, tok in enumerate(pending):
                j = k * len(rows) // len(pending)
                rows[j] = jnp.where(never, tok, rows[j])
            pending.clear()
            u = jnp.concatenate(rows, axis=0)
        return pltpu.bitcast(u, BF16)

    def dot(lhs_words, rhs):
        a = jnp.concatenate([tied(u) for u in lhs_words], axis=1)[:, :rhs.shape[0]]
        r = jnp.dot(a, rhs, preferred_element_type=F32)
        begin = issued[-1][1] if issued else 0
        issued.append((begin, begin + a.shape[0] * len(lhs_words) // 4, r))
        return r

    @_memo
    def lane_after(n):
        iota = lax.broadcasted_iota(jnp.int32, (8, L), 1)
        return iota if n < 0 else jnp.where(never, pltpu.bitcast(issued[n][2][:8], jnp.int32), iota)

    def lane():
        return lane_after(sum(e[0] <= issued[-1][1] - LEAD for e in issued) - 1)

    def pack(ref, idx, v):
        ref[idx] = v.astype(BF16)
        return ref.bitcast(U32)[idx]

    def colsum(f):
        @_memo
        def part(k):
            return _tree(jnp.add, _vregs(f(slice(k * RP, (k + 1) * RP))) + ([part(k - 1)] if k else []))
        total = _memo(lambda: jnp.sum(part(D // RP - 1), axis=0, keepdims=True))
        return total, [P(lambda k: anchor(part(k)), k) for k in range(D // RP - 1)]

    def anchor_row(f):
        anchor(jnp.broadcast_to(f(), (8, L)))

    mod_sum = _memo(lambda t: colsum(lambda rs: load(wm_v, _MOD_CUTS, rs, t).astype(F32) * silu_c[rs]))
    mod_tile = _memo(lambda t: _cols(mod_sum(t)[0]()))

    @_memo
    def mod(i):
        t0 = i * D // L
        m = jnp.concatenate([mod_tile(t) for t in range(t0, t0 + 5)], axis=0)[i * D - t0 * L:][:D]
        m = 1.0 + m if i in (1, 4) else m
        return GA * m if i in (3, 4) else m

    def layernorm(x, scale, shift):
        s1, units1 = colsum(lambda rs: x()[rs])
        mean = _memo(lambda: s1() * (1.0 / D))
        s2, units2 = colsum(lambda rs: jnp.square(x()[rs] - mean()))
        neg_rstd = _memo(lambda: -lax.rsqrt(s2() * (1.0 / D) + EPS))
        out = _memo(lambda: (mean() - x()) * neg_rstd() * mod(scale) + mod(shift))
        return out, units1 + [P(anchor_row, mean)] + units2 + [P(anchor_row, neg_rstd)]

    x_tile = _memo(lambda t: load(x_v, _X_CUTS, slice(None), t).astype(F32))
    ln1 = _memo(lambda t: layernorm(P(x_tile, t), 1, 0))
    h1 = _memo(lambda t: pack(h1_s, t, ln1(t)[0]()))

    @_memo
    def wqkv_tile(kt, nt):
        nr = min(L, D - kt * L)
        blk = load(wqkv_v, _QKV_CUTS, pl.ds(kt * L, nr), nt)
        if nr < L:
            blk = jnp.concatenate([blk, jnp.zeros((L - nr, blk.shape[1]), BF16)], axis=0)
        wt32[kt, pl.ds(nt * L, blk.shape[1])] = blk.T.astype(F32)

    @_memo
    def wqkv_t(pg, kt):
        for nt in range(pg * R // L, ((pg + 1) * R - 1) // L + 1):
            wqkv_tile(kt, nt)
        return pack(wqkv_s, (pg, kt), jnp.concatenate(
            [wt32[kt, pl.ds(pg * R + d, 8, stride=DH), :] for d in range(DH)], axis=0))

    qkv = _memo(lambda p, g, t: dot([wqkv_t(p * G + g, kt) for kt in range(5)],
                                    pltpu.bitcast(h1(t), BF16)))
    row = _memo(lambda p, g, t, d: qkv(p, g, t)[d * 8:(d + 1) * 8])

    def back(prev, cur, sh):
        return pltpu.roll(cur if prev is cur else jnp.where(lane() >= L - sh, prev, cur), sh, 1)

    def ahead(cur, nxt, sh):
        return pltpu.roll(jnp.where(lane() < sh, nxt, cur), L - sh, 1)

    @_memo
    def scores(t, g, d):
        q = row(0, g, t, d)
        qs = (q, ahead(q, row(0, g, min(t + 1, NT - 1), d), GS))
        k = row(1, g, t, d)
        ks = [k] + [back(row(1, g, max(t - 1, 0), d), k, b * DIL) for b in range(1, HW)]
        prod = [q * k for q in qs for k in ks]
        return prod if d == 0 else [a + b for a, b in zip(scores(t, g, d - 1), prod)]

    @_memo
    def probs(t, g):
        cur, prev = scores(t, g, DH - 1), scores(max(t - 1, 0), g, DH - 1)
        lg = cur[:HW] + [back(prev[w], cur[w], GS) for w in range(HW, W)]
        if t == 0:
            lg = [jnp.where(lane() >= w * DIL, v, -1e9 * DH ** 0.5) for w, v in enumerate(lg)]
        mx = functools.reduce(jnp.maximum, lg)
        e = [jnp.exp2((v - mx) * (DH ** -0.5 / math.log(2.0))) for v in lg]
        inv = 1.0 / functools.reduce(jnp.add, e)
        return [v * inv for v in e]

    @_memo
    def probs_far(t, g):
        if t < 0:
            return pltpu.roll(functools.reduce(jnp.add, probs(0, g)[HW:]), L - GS, 1)
        return [ahead(probs(t, g)[w], probs(min(t + 1, NT - 1), g)[w], GS) for w in range(HW, W)]

    v_first = _memo(lambda g, d: jnp.broadcast_to(row(2, g, 0, d)[:, 0:1], (8, L)))

    @_memo
    def mixed(t, g, d):
        if t < 0:
            return None, probs_far(t, g) * v_first(g, d)
        v = row(2, g, t, d)
        vs = [v] + [back(row(2, g, t - 1, d) if t else v_first(g, d), v, b * DIL) for b in range(1, HW)]
        return tuple(functools.reduce(jnp.add, [a * v for a, v in zip(p, vs)])
                     for p in (probs(t, g)[:HW], probs_far(t, g)))

    @_memo
    def attn(t, g, d0):
        return pack(o_s, (t, (g * DH + d0) // DU), jnp.concatenate(
            [mixed(t, g, d)[0] + back(mixed(t - 1, g, d)[1], mixed(t, g, d)[1], GS)
             for d in range(d0, d0 + DU)], axis=0))

    def attn_units(n):
        def at(lag, ds=(0,)):
            return [divmod(n - lag, G) + (d,) for d in ds] if 0 <= n - lag < NT * G else []
        ds = range(0, DH, DU)
        return _merge(
            [P(lambda t, g, d: anchor(*scores(t, g, d + DU - 1)), *a) for a in at(0, ds)],
            [P(lambda t, g, d: anchor(*probs(t, g)), *a) for a in at(ATT_LAG[0])],
            [P(lambda t, g, d: anchor(*probs_far(t, g)), *a) for a in at(G + ATT_LAG[1])],
            [P(lambda t, g, d: anchor(*[v for e in range(d, d + DU) for v in mixed(t, g, e)]), *a)
             for a in at(G + ATT_LAG[2], ds)],
            [P(lambda *a: anchor(attn(*a)), *a) for a in at(G + ATT_LAG[3], ds)])

    @_memo
    def wo_rows(nt, g):
        blk = wo_v[pl.ds(g * R, R), pl.ds(nt * L, min(L, D - nt * L))].astype(F32)
        if blk.shape[1] < L:
            blk = jnp.concatenate([blk, jnp.zeros((R, L - blk.shape[1]), F32)], axis=1)
        wo32[nt, pl.ds(g * R, R)] = blk

    @_memo
    def wo_t(nt, kt):
        def rows(g, d):
            if g >= G:
                return jnp.zeros((8, L), F32)
            wo_rows(nt, g)
            return wo32[nt, pl.ds(g * R + d, 8, stride=DH), :]
        blk = jnp.concatenate([rows(*divmod(16 * kt + j, DH)) for j in range(16)], axis=0)
        return pack(wo_s, (nt, kt), blk.astype(BF16).T)[:min(L, D - nt * L) // 2]

    wo_all = _memo(lambda kt: jnp.concatenate([wo_t(nt, kt) for nt in range(5)], axis=0))
    attn_all = _memo(lambda t: pltpu.bitcast(jnp.concatenate(
        [attn(t, g, d) for g in range(G) for d in range(0, DH, DU)], axis=0), BF16))
    proj = _memo(lambda g, t: dot([wo_all(kt)[g * R // 2:(g + 1) * R // 2] for kt in range(5)],
                                  attn_all(t)))
    x2 = _memo(lambda t: x_tile(t) + mod(2) * jnp.concatenate([proj(g, t) for g in range(G)], axis=0))
    ln2 = _memo(lambda t: layernorm(P(x2, t), 4, 3))

    def operand_units(words, order, n):
        tok = _memo(lambda o: token(*words(o).values()))
        return [P(lambda o, r: pending.append(tok(o)[r:r + 8]), o, r)
                for o in order for r in range(0, n // 2, 8)]

    order_a, order_b = (1, 5, 0, 2, 3, 4, 6), (6, 3, 0, 1, 4, 5, 2)
    h_rem = _memo(lambda t: pack(hr_s, t, ln2(t)[0]()[4 * L:]))
    h_outer = _memo(lambda b: _outer(_SB, lambda r, j: ln2(4 * b + j)[0]()[r * L:(r + 1) * L]))

    @_memo
    def h_words(b, o):
        def operand(i):
            if o not in _REM:
                return _comb(_SB[i], P(h_outer(b), o))
            low = _comb(_SB[i], lambda qi: h_outer(b)(o, qi)[:L // 2])
            high = _comb(_SB[i], lambda qi: h_outer(b)(o, qi ^ 1)[L // 2:])
            return jnp.concatenate([low, -high if i in (1, 4) else high], axis=0)
        return {i: pack(hc_s, (b, 7 * o + i), operand(i)) for i in order_b}

    @_memo
    def up_rhs(b, o, i):
        a = h_words(b, o)
        if o not in _REM:
            return pltpu.bitcast(a[i], BF16)
        zero = jnp.zeros((L // 4, L), U32)
        rem = [h_rem(4 * b + 2 * _REM[o][1] + j) for j in range(2)]
        low = {7: zero, 8: rem[0], 9: rem[1]}[i] if i > 6 else a[i][:L // 4]
        high = ({0: zero, 5: rem[1], 6: rem[0]}[i] if i in (0, 5, 6)
                else a[{2: 3, 3: 2, 7: 0, 8: 5, 9: 6}.get(i, i)][L // 4:])
        return pltpu.bitcast(jnp.concatenate([low, high], axis=0), BF16)

    @_memo
    def w1_t(c, r, k):
        u = pltpu.bitcast(w1_v[pl.ds(k * L, min(L, D - k * L)), pl.ds((4 * c + r) * L, L)], U32)
        u = [jnp.where(never, pltpu.bitcast(lane(), U32), u[:8]), u[8:]]
        return pltpu.bitcast(jnp.concatenate(u * (1 + k // 4), axis=0), BF16).T.astype(F32)

    b1 = _memo(lambda: b1_v[...].astype(F32))
    b1_col = _memo(lambda c, r: _cols(GA * b1()[4 * c + r:][:1]))
    w1_outer = _memo(lambda c: _outer(_SA, P(w1_t, c)))
    low_lanes = lax.broadcasted_iota(jnp.int32, (L // 2, L), 1) < L // 2

    @_memo
    def w1_words(c, o):
        a = {i: pack(w1c_s, (c, 7 * o + i), _comb(_SA[i], P(w1_outer(c), o))) for i in order_a}
        if o in _REM:
            rem = [pack(w1r_s, (c, 2 * o + ri), _comb(_REM[o][0], lambda ro: w1_t(c, 2 * ro + ri, 4)))
                   for ri in range(2)]
            a.update({i: jnp.where(low_lanes, low, high) for i, low, high in (
                (2, a[2], a[3]), (3, a[3], a[2]), (5, a[5], rem[1]), (6, a[6], rem[0]),
                (8, rem[1], a[5]), (9, rem[0], a[6]))})
        return a

    w2_outer = _memo(lambda c: _outer(
        _SA, lambda r, k: w2t_v[pl.ds(r * R, R), pl.ds((4 * c + k) * L, L)].astype(F32)))
    w2_words = _memo(lambda c, o: {
        i: pack(w2c_s, (c, 7 * o + i), _comb(_SA[i], P(w2_outer(c), o))) for i in order_a})

    up = _memo(lambda b, c, o, i: dot([w1_words(c, o)[0 if i == 7 else i]], up_rhs(b, o, i)))

    @_memo
    def up_inner(b, c, o, qi):
        v = _result(qi, P(up, b, c, o))
        return v + (up(b, c, o, 7) + up(b, c, o, 10 - qi)) if o in _REM and qi in (1, 2) else v

    def hidden(b, c, r, j):
        w = _result(r // 2 * 2 + j // 2, lambda o: up_inner(b, c, o, r % 2 * 2 + j % 2)) + b1_col(c, r)
        return w + w * jnp.tanh(w * (_C / GA + w * w))

    g_outer = _memo(lambda b, c: _outer(_SB, P(hidden, b, c)))
    g_token = _memo(lambda b, c, qi: token(*[g_outer(b, c)(o, qi) for o in (0, 2, 3, 5, 6)]))
    chunks = [range(sum(SPANS[:k]), sum(SPANS[:k + 1])) for k in range(len(SPANS))]

    @_memo
    def down(b, k, o, i):
        rhs = jnp.concatenate([_comb(_SB[i], P(g_outer(b, c), o)) for c in chunks[k]], axis=0)
        y = dot([w2_words(c, o)[i] for c in chunks[k]], rhs.astype(BF16))
        if k == 0:
            return y
        acc = down(b, k - 1, o, i)
        return jnp.concatenate([y[:16] + acc[:16], y[16:] + acc[16:]], axis=0)

    b2_col = _memo(lambda: column(b2_v[...].astype(F32).reshape(1, D)))
    gate = _memo(lambda: (0.5 / GA * mod(5), mod(5) * b2_col()))
    down_inner = _memo(lambda b, o, qi: _result(qi, P(down, b, len(SPANS) - 1, o)))

    @_memo
    def out_block(b, qo, qi):
        r, j = _rc(qo, qi)
        rs = slice(r * R, (r + 1) * R)
        y = _result(qo, lambda o: down_inner(b, o, qi))
        return pack(out_v, 4 * (4 * b + j) + r, (x2(4 * b + j)[rs] + gate()[1][rs]) + gate()[0][rs] * y)

    def write_back(b, qo):
        for qi in range(4):
            out_block(b, qo, qi)
        for qi in range(4):
            r, j = _rc(qo, qi)
            pltpu.make_async_copy(out_v.at[4 * (4 * b + j) + r],
                                  out_hbm.at[pl.ds(r * R, R), pl.ds((4 * b + j) * L, L)], out_sem).start()

    order = [(p, t) for p in range(2) for t in range(X0)] + [(2, 0), (0, X0), (2, 1)]
    for t in range(X0, NT + 2):
        order += [e for e in ((0, t + 1), (1, t), (2, t - 2)) if e[1] < NT]
        order += [(3, t - PROJ_FROM)] * (0 <= t - PROJ_FROM < PROJ_EARLY)
    when = {e: k / 4 for k, e in enumerate(order)}
    att = []
    for t in range(NT + 3):
        ready = [when[1, min(t, NT - 1)] + 0.3249, when[0, min(t + 1, NT - 1)] + 0.3249]
        ready += [when[2, min(t - 2, NT - 1)] + 0.075] if t >= 2 else []
        att.append(max(ready + [a + ATT_STEP[(t > 2) + (t > NT)] for a in att[-1:]]))
    att.append(att[-1] + 0.2)
    for t in range(PROJ_EARLY, NT):
        when[3, t] = max(max(when.values()) + 0.25, att[t + 4])
    arrive = (when[0, 2], when[1, 2], T_WAVE3, T_WAVE4)
    assert when[0, X1 - 1] >= T_WAVE3 and all(when[3, t] >= att[t + 4] for t in range(NT))
    items = [(t, P(wait, ds)) for t, ds in zip(arrive, waves)]
    items += [(t, P(start, ds)) for t, ds in zip((0,) + arrive[1:], waves[1:])]

    def spread(fs, t0, t1, vector=True):
        for j, f in enumerate(fs):
            t = t0 + (t1 - t0) * (j + 0.5) / len(fs)
            for tb in arrive:
                if vector and tb <= t < min(tb + 0.5, t1):
                    t = tb + 0.3 * min(0.5, t1 - tb) + 0.7 * (t - tb)
            items.append((t, f))

    for (p, t), s in when.items():
        spread([P(qkv, p, g, t) if p < 3 else P(proj, g, t) for g in range(G)],
               s, s + (0.25 if s < T_MLP else 1e-3), False)
    stats_end, h2_end = [T_WAVE3 + 1 + 0.4 * T_MOD], [T_WAVE3 + 1 + T_MOD]
    for t in range(NT):
        if t:
            spread(ln1(t)[1] + [P(lambda t, r: anchor(h1(t)[r:r + 24]), t, r) for r in range(0, D // 2, 24)],
                   when[1, 3] if t == X0 else when[0, t - 1], when[0, t])
        stats_end.append(max(when[3, t] + 0.25, stats_end[-1]) + T_LN)
        spread(ln2(t)[1], stats_end[-1] - T_LN, stats_end[-1])
        h2_end.append(max(stats_end[-1], h2_end[-1]) + T_LN)
        spread([P(lambda t, r: anchor(ln2(t)[0]()[r:r + 32]), t, r) for r in range(0, 4 * L, 32)]
               + [P(lambda t: anchor(h_rem(t)), t)], h2_end[-1] - T_LN, h2_end[-1])
    for p in (1, 2):
        spread([P(lambda *a: anchor(wqkv_t(*a)), p * G + g, kt) for g in range(G) for kt in range(5)],
               arrive[p - 1], when[p, 0])
    for t in range(NT + 3):
        spread(sum([attn_units(t * G + g) for g in range(G)], []), att[t], att[t + 1])
    spread([P(lambda *a: anchor(wo_t(*a)), nt, kt) for nt in range(5) for kt in range(5)],
           T_WAVE3, when[3, 0])
    for tiles, t0, t1 in ((range(9, 23), T_WAVE3 + 0.5, T_WAVE3 + 0.5 + T_MOD),
                          (range(23, 27), T_MLP + 21, T_MLP + 25)):
        spread(sum([mod_sum(t)[1] + [P(anchor_row, mod_sum(t)[0])] for t in tiles], []), t0, t1)
        spread([P(lambda t: anchor(mod_tile(t)), t) for t in tiles], t0 + 0.4, t1 + 0.4)
    spread([lambda: anchor(b2_col())], T_MLP + 25, T_MLP + 26)

    jobs = [(b, k) for k in range(len(SPANS)) for b in range(NB)]
    up_at = {bc: T_MLP + s for s, bc in enumerate((b, c) for b, k in jobs for c in chunks[k])}
    down_at = [up_at[b, chunks[k][-1]] + 2 for b, k in jobs]
    down_at.append(down_at[-1] + SPANS[-1])
    for n in range(len(jobs) - 2, 0, -1):
        gap = down_at[n + 1] - down_at[n - 1] - SPANS[jobs[n][1]] - SPANS[jobs[n - 1][1]]
        down_at[n] = max(down_at[n], down_at[n + 1] - SPANS[jobs[n][1]] - gap / 2.0)

    prep = [(up_at[b, 0], h2_end[4 * b + 4], [], operand_units(P(h_words, b), order_b, L))
            for b in range(NB)]
    for k, cs in enumerate(chunks):
        for c in cs:
            xpose = [P(lambda c, r, n: anchor(w1_t(c, r, n)[:8] if n < 5 else b1_col(c, r)), c, r, n)
                     for r in range(4) for n in range(6)]
            prep.append((up_at[0, c], T_WAVE4 + 1, xpose, operand_units(P(w1_words, c), order_a, L)))
            prep.append((down_at[NB * k], T_WAVE4, [], operand_units(P(w2_words, c), order_a, R)))
    prep.sort(key=lambda e: e[:2])
    now, step = T_PREP, 1.0
    while prep:
        now = max(now, min(e[1] for e in prep))
        k = min(k for k, e in enumerate(prep) if e[1] <= now)
        last, step = step, min((e[0] - now) / (j + 1 + (j < k)) for j, e in enumerate(prep))
        _, _, xpose, units = prep.pop(k)
        spread(xpose, now - min(last, 1.0), now)
        spread(units, now, now + step)
        now += step

    def last_down(n):
        down(*jobs[-1], *_DOWN[n])
        for qo, done in _DONE.items():
            if n == done + 2:
                tok = token(*[out_block(NB - 1, qo, qi) for qi in range(4)])
                pending.extend(_vregs(tok))
            if n == min(done + 4, len(_DOWN) - 1):
                write_back(NB - 1, qo)

    def rounds(fs, n):
        return [P(lambda fs: [f() for f in fs], fs[j:j + n]) for j in range(0, len(fs), n)]

    spread(rounds([P(up, b, c, o, i) for b, c in up_at for o, i in _UP], 4),
           T_MLP - 0.1, T_MLP + len(up_at) - 0.1, False)
    for n, (b, k) in enumerate(jobs):
        fs = [P(last_down, m) if (b, k) == jobs[-1] else P(down, b, k, *oi) for m, oi in enumerate(_DOWN)]
        spread(rounds(fs, max(1, 4 // SPANS[k])), down_at[n], down_at[n + 1], False)
    for (b, c), s in up_at.items():
        spread([P(lambda b, c, qi, r: pending.append(g_token(b, c, qi)[r:r + 8]), b, c, qi, r)
                for r in range(0, L, 8) for qi in (0, 2, 3, 1)], s + 1, s + 2)
    for b in range(NB - 1):
        s = down_at[b - NB]
        spread([P(lambda b, qi, r: anchor(*[out_block(b, qo, qi)[r:r + 8] for qo in range(4)]), b, qi, r)
                for r in range(0, R // 2, 8) for qi in range(4)], s + 0.1, s + 3)
        spread([P(write_back, b, qo) for qo in range(4)], s + 3.2, s + 3.5, False)

    d_m0.wait()
    mod(0)
    d_m1.wait()
    mod(1)
    d_wq.wait()
    start(waves[0])
    for g in range(G):
        for kt in range(5):
            wqkv_t(g, kt)
    d_x0.wait()
    for _, f in sorted(items, key=lambda e: e[0]):
        f()
    pltpu.make_async_copy(out_v, out_v, out_sem).wait()


@jax.jit
def pallas_adaLN_cond__sliding_local_dilated__dense_activation_gelu__prompt_kernel(
    A_x: jax.Array,
    A_wqkv: jax.Array,
    A_wo: jax.Array,
    B_x: jax.Array,
    B_w1: jax.Array,
    B_b1: jax.Array,
    B_w2: jax.Array,
    B_b2: jax.Array,
    c: jax.Array,
    w_mod: jax.Array,
):
    del B_x

    def pieces(cuts):
        return [pltpu.VMEM((D, b - a), BF16) for a, b in zip(cuts, cuts[1:])]

    scratch = [
        pieces(_X_CUTS), pieces(_QKV_CUTS), pieces(_MOD_CUTS),
        pltpu.VMEM((D, D), BF16),
        pltpu.VMEM((D, F), BF16),
        pltpu.VMEM((F // L, L), BF16),
        pltpu.VMEM((D, F), BF16),
        pltpu.VMEM((D,), BF16),
        pltpu.VMEM((1, D), BF16),
        pltpu.VMEM((5, 3 * D, L), F32),
        pltpu.VMEM((5, D, L), F32),
        pltpu.VMEM((3 * G, 5, R, L), BF16),
        pltpu.VMEM((5, 5, L, L), BF16),
        pltpu.VMEM((NT, D, L), BF16),
        pltpu.VMEM((NT, G * DH // DU, DU * 8, L), BF16),
        pltpu.VMEM((NB, 49, L, L), BF16),
        pltpu.VMEM((NT, L // 2, L), BF16),
        pltpu.VMEM((NC, 49, L, L), BF16),
        pltpu.VMEM((NC, 14, L, L), BF16),
        pltpu.VMEM((NC, 49, R, L), BF16),
        pltpu.VMEM((4 * NT, R, L), BF16),
        pltpu.SemaphoreType.DMA((17,)),
        pltpu.SemaphoreType.DMA(()),
    ]
    hbm = pl.BlockSpec(memory_space=pl.ANY)
    out_t = pl.pallas_call(
        _kernel,
        out_shape=jax.ShapeDtypeStruct((D, S), BF16),
        in_specs=[hbm] * 9,
        out_specs=hbm,
        scratch_shapes=scratch,
        compiler_params=pltpu.CompilerParams(vmem_limit_bytes=126 * 2**20),
    )(A_x[0].T, A_wqkv, A_wo, B_w1, B_b1.reshape(F // L, L), B_w2.T, B_b2, c, w_mod)
    return out_t.T[None]
```

```python
import functools
import math

import jax
import jax.numpy as jnp
from jax import lax
import jax.experimental.pallas as pl
import jax.experimental.pallas.tpu as pltpu

F32, BF16, U32 = jnp.float32, jnp.bfloat16, jnp.uint32
P = functools.partial
_memo = functools.lru_cache(maxsize=None)

S, D, F = 2048, 576, 4608
DH, W, DIL = 18, 8, 2
EPS = 1e-5
L = 128
NT = S // L
G = 4
R = D // G
NB = NT // 4
NC = F // (4 * L)
HW = W // 2
GS = HW * DIL

X0, X1 = 4, 8
T_WAVE3, T_WAVE4 = 4.25, 12.25
T_MOD, T_LN, T_PREP, T_MLP = 5.0, 0.5, 14.0, 16.0
ATT_STEP = (0.55, 0.85, 0.4)
ATT_LAG = (2, 4, 5, 7)
PROJ_FROM, PROJ_EARLY = 8, 9
SPANS = (2, 3, 4)
LEAD = 810
DU = 6
RP = D // 6

_SA = (((0, 1), (3, 1)), ((2, 1), (3, 1)), ((0, 1),), ((3, 1),),
       ((0, 1), (1, 1)), ((2, 1), (0, -1)), ((1, 1), (3, -1)))
_SB = (((0, 1), (3, 1)), ((0, 1),), ((1, 1), (3, -1)), ((2, 1), (0, -1)),
       ((3, 1),), ((0, 1), (1, 1)), ((2, 1), (3, 1)))
_REM = {2: (((0, 1),), 1), 3: (((1, 1),), 0), 5: (((1, 1), (0, -1)), 1), 6: (((0, 1), (1, -1)), 0)}
_OUTER = (1, 3, 2, 4, 0, 6, 5)
_UP = [(o, i) for o in _OUTER for i in (0, 1, 3, 6, 2, 4, 5, 7, 9, 8) if i < 7 or o in _REM]
_DOWN = [(o, i) for o in _OUTER for i in (0, 1, 3, 6, 2, 4, 5)]
_DONE = {qo: 7 * max(map(_OUTER.index, need)) + 6
         for qo, need in enumerate(((0, 3, 4, 6), (2, 4), (1, 3), (0, 1, 2, 5)))}

_C = math.sqrt(2.0 / math.pi)
GA = (0.044715 * _C) ** (1.0 / 3.0)


def _comb(terms, get):
    r = None
    for i, s in terms:
        r = get(i) if r is None else (r + get(i) if s > 0 else r - get(i))
    return r


def _result(q, m):
    if q == 0:
        return ((m(0) + m(3)) + m(6)) - m(4)
    if q == 3:
        return (m(0) - m(1)) + (m(2) + m(5))
    return m(2) + m(4) if q == 1 else m(1) + m(3)


def _rc(qo, qi):
    return 2 * (qo // 2) + qi // 2, 2 * (qo % 2) + qi % 2


def _outer(tab, block):
    block = _memo(block)
    return _memo(lambda o, qi: _comb(tab[o], lambda qo: block(*_rc(qo, qi))))


def _tree(op, vals):
    vals = list(vals)
    while len(vals) > 1:
        vals = [op(a, b) for a, b in zip(vals[::2], vals[1::2])] + vals[len(vals) & ~1:]
    return vals[0]


def _fold(op, v):
    rest = []
    while v.shape[0] > 8:
        h = v.shape[0] // 16 * 8
        rest += [v[2 * h:]] if v.shape[0] > 2 * h else []
        v = op(v[:h], v[h:2 * h])
    return functools.reduce(op, rest, v)


def _cols(row):
    return jnp.broadcast_to(row, (L, row.shape[1])).astype(BF16).T.astype(F32)


def _merge(*streams):
    out = [((j + 0.5) / len(st), k, f) for k, st in enumerate(streams) for j, f in enumerate(st)]
    return [e[2] for e in sorted(out, key=lambda e: e[:2])]


_X_CUTS = (0, (X0 - 1) * L, X0 * L, X1 * L, S)
_QKV_CUTS = (0, 5 * L, 9 * L, 3 * D)
_MOD_CUTS = (0, 5 * L, 9 * L, 23 * L, 6 * D)


def _kernel(x_hbm, wqkv_hbm, wo_hbm, w1_hbm, b1_hbm, w2t_hbm, b2_hbm, c_hbm, wm_hbm, out_hbm,
            x_v, wqkv_v, wm_v, wo_v, w1_v, b1_v, w2t_v, b2_v, c_v,
            wt32, wo32, wqkv_s, wo_s, h1_s, o_s, hc_s, hr_s, w1c_s, w1r_s, w2c_s, out_v,
            sems, out_sem):
    srcs = [(c_hbm, c_v), (wo_hbm, wo_v), (w1_hbm, w1_v), (w2t_hbm, w2t_v), (b1_hbm, b1_v),
            (b2_hbm, b2_v)]
    for hbm, bufs, cuts in ((x_hbm, x_v, _X_CUTS), (wqkv_hbm, wqkv_v, _QKV_CUTS),
                            (wm_hbm, wm_v, _MOD_CUTS)):
        srcs += [(hbm.at[:, pl.ds(a, b - a)], buf) for buf, a, b in zip(bufs, cuts, cuts[1:])]
    (d_c, d_wo, d_w1, d_w2, d_b1, d_b2, d_x0, d_x1, d_x2, d_x3, d_wq, d_wk, d_wv,
     d_m0, d_m1, d_m2, d_m3) = [
        pltpu.make_async_copy(src, dst, sems.at[k]) for k, (src, dst) in enumerate(srcs)]
    waves = ([d_wk, d_x1], [d_wv, d_x2], [d_x3, d_wo, d_m2], [d_w1, d_w2, d_m3, d_b1, d_b2])

    def start(ds):
        for d in ds:
            d.start()

    def wait(ds):
        for d in ds:
            d.wait()

    def load(bufs, cuts, rows, tile):
        k = max(k for k, a in enumerate(cuts) if a <= tile * L)
        return bufs[k][rows, pl.ds(tile * L - cuts[k], min(L, cuts[-1] - tile * L))]

    def column(row):
        return _cols(jnp.concatenate([row, jnp.zeros((1, 5 * L - D), F32)], axis=1))[:D]

    start([d_c, d_m0, d_m1, d_wq, d_x0])
    d_c.wait()
    c = c_v[...].astype(F32)
    silu_c = column(c * jax.nn.sigmoid(c))

    never = jnp.abs(silu_c[:8]) < 0.0
    pending, issued = [], []

    def token(*vals):
        return _tree(jnp.bitwise_or, [v if v.dtype == U32 else pltpu.bitcast(v, U32) for v in vals])

    def anchor(*vals):
        pending.append(_fold(jnp.bitwise_or, token(*vals)))

    def tied(u):
        if pending:
            parts, end = [], 0
            for k, tok in enumerate(pending):
                r = k * (u.shape[0] // 8) // len(pending) * 8
                if r >= end:
                    parts += ([u[end:r]] if r > end else []) + [u[r:r + 8]]
                    end = r + 8
                parts[-1] = lax.select(never, tok, parts[-1])
            pending.clear()
            u = jnp.concatenate(parts + ([u[end:]] if end < u.shape[0] else []), axis=0)
        return pltpu.bitcast(u, BF16)

    def dot(lhs_words, rhs):
        a = jnp.concatenate([tied(u) for u in lhs_words], axis=1)[:, :rhs.shape[0]]
        r = jnp.dot(a, rhs, preferred_element_type=F32)
        begin = issued[-1][1] if issued else 0
        issued.append((begin, begin + a.shape[0] * len(lhs_words) // 4, r))
        return r

    @_memo
    def lane_after(n):
        iota = lax.broadcasted_iota(jnp.int32, (8, L), 1)
        return iota if n < 0 else lax.select(never, pltpu.bitcast(issued[n][2][:8], jnp.int32), iota)

    def recent():
        return sum(e[0] <= issued[-1][1] - LEAD for e in issued) - 1

    lanes_from = _memo(lambda n, first, rows: jnp.concatenate([lane_after(n)] * (rows // 8), axis=0) >= first)

    def pack(ref, idx, v):
        ref[idx] = v.astype(BF16)
        return ref.bitcast(U32)[idx]

    def colsum(f):
        @_memo
        def part(k):
            v = _fold(jnp.add, f(slice(k * RP, (k + 1) * RP)))
            return v + part(k - 1) if k else v
        total = _memo(lambda: jnp.sum(part(D // RP - 1), axis=0, keepdims=True))
        return total, [P(lambda k: anchor(part(k)), k) for k in range(D // RP - 1)]

    def anchor_row(f):
        anchor(jnp.broadcast_to(f(), (8, L)))

    mod_sum = _memo(lambda t: colsum(lambda rs: load(wm_v, _MOD_CUTS, rs, t).astype(F32) * silu_c[rs]))
    mod_tile = _memo(lambda t: _cols(mod_sum(t)[0]()))

    @_memo
    def mod(i):
        t0 = i * D // L
        m = jnp.concatenate([mod_tile(t) for t in range(t0, t0 + 5)], axis=0)[i * D - t0 * L:][:D]
        m = 1.0 + m if i in (1, 4) else m
        return GA * m if i in (3, 4) else m

    def layernorm(x, scale, shift):
        s1, units1 = colsum(lambda rs: x()[rs])
        mean = _memo(lambda: s1() * (1.0 / D))
        s2, units2 = colsum(lambda rs: jnp.square(x()[rs] - mean()))
        neg_rstd = _memo(lambda: -lax.rsqrt(s2() * (1.0 / D) + EPS))
        out = _memo(lambda: (mean() - x()) * neg_rstd() * mod(scale) + mod(shift))
        return out, units1 + [P(anchor_row, mean)] + units2 + [P(anchor_row, neg_rstd)]

    x_tile = _memo(lambda t: load(x_v, _X_CUTS, slice(None), t).astype(F32))
    ln1 = _memo(lambda t: layernorm(P(x_tile, t), 1, 0))
    h1 = _memo(lambda t: pack(h1_s, t, ln1(t)[0]()))

    @_memo
    def wqkv_tile(kt, nt):
        nr = min(L, D - kt * L)
        blk = load(wqkv_v, _QKV_CUTS, pl.ds(kt * L, nr), nt)
        if nr < L:
            blk = jnp.concatenate([blk, jnp.zeros((L - nr, blk.shape[1]), BF16)], axis=0)
        wt32[kt, pl.ds(nt * L, blk.shape[1])] = blk.T.astype(F32)

    @_memo
    def wqkv_t(pg, kt):
        for nt in range(pg * R // L, ((pg + 1) * R - 1) // L + 1):
            wqkv_tile(kt, nt)
        return pack(wqkv_s, (pg, kt), jnp.concatenate(
            [wt32[kt, pl.ds(pg * R + d, 8, stride=DH), :] for d in range(DH)], axis=0))

    qkv = _memo(lambda p, g, t: dot([wqkv_t(p * G + g, kt) for kt in range(5)],
                                    pltpu.bitcast(h1(t), BF16)))
    dims = _memo(lambda p, g, t, d: qkv(p, g, t)[d * 8:(d + DU) * 8])

    def back(prev, cur, sh):
        if prev is not cur:
            cur = lax.select(lanes_from(recent(), L - sh, cur.shape[0]), prev, cur)
        return pltpu.roll(cur, sh, 1)

    def ahead(cur, nxt, sh):
        return back(cur, nxt, L - sh)

    @_memo
    def scores(t, g, d):
        q = dims(0, g, t, d)
        qs = (q, ahead(q, dims(0, g, min(t + 1, NT - 1), d), GS))
        k = dims(1, g, t, d)
        ks = [k] + [back(dims(1, g, max(t - 1, 0), d), k, b * DIL) for b in range(1, HW)]
        part = [jnp.sum((q * k).reshape(DU, 8, L), axis=0) for q in qs for k in ks]
        return [a + b for a, b in zip(scores(t, g, d - DU), part)] if d else part

    @_memo
    def probs(t, g):
        cur, prev = scores(t, g, DH - DU), scores(max(t - 1, 0), g, DH - DU)
        lg = cur[:HW] + [back(prev[w], cur[w], GS) for w in range(HW, W)]
        if t == 0:
            lg = [jnp.where(lanes_from(-1, w * DIL, 8), v, -1e9 * DH ** 0.5) for w, v in enumerate(lg)]
        lg = jnp.stack(lg)
        e = jnp.exp2((lg - jnp.max(lg, axis=0)) * (DH ** -0.5 / math.log(2.0)))
        p = (e * (1.0 / jnp.sum(e, axis=0))).reshape(W * 8, L)
        return p[:HW * 8], p[HW * 8:]

    probs_far = _memo(lambda t, g: ahead(probs(max(t, 0), g)[1], probs(min(t + 1, NT - 1), g)[1], GS))
    weights = _memo(lambda t, g, far: [
        jnp.concatenate([(probs_far(t, g) if far else probs(t, g)[0])[8 * b:8 * b + 8]] * DU, axis=0)
        for b in range(HW)])
    v_first = _memo(lambda g, d: jnp.broadcast_to(dims(2, g, 0, d)[:, 0:1], (DU * 8, L)))

    @_memo
    def mixed(t, g, d):
        if t < 0:
            return None, functools.reduce(jnp.add, weights(t, g, 1)) * v_first(g, d)
        v = dims(2, g, t, d)
        vs = [v] + [back(dims(2, g, t - 1, d) if t else v_first(g, d), v, b * DIL) for b in range(1, HW)]
        return [functools.reduce(jnp.add, [a * v for a, v in zip(weights(t, g, far), vs)])
                for far in range(2)]

    attn = _memo(lambda t, g, d: pack(o_s, (t, (g * DH + d) // DU), mixed(t, g, d)[0] + back(
        mixed(t - 1, g, d)[1], mixed(t, g, d)[1], GS)))

    def attn_units(n):
        def at(lag, ds=(0,)):
            return [divmod(n - lag, G) + (d,) for d in ds] if 0 <= n - lag < NT * G else []
        ds = range(0, DH, DU)
        return _merge(
            [P(lambda *a: anchor(*scores(*a)), *a) for a in at(0, ds)],
            [P(lambda t, g, d: anchor(*probs(t, g)), *a) for a in at(ATT_LAG[0])],
            [P(lambda t, g, d: anchor(probs_far(t, g)), *a) for a in at(G + ATT_LAG[1])],
            [P(lambda *a: anchor(*mixed(*a)), *a) for a in at(G + ATT_LAG[2], ds)],
            [P(lambda *a: anchor(attn(*a)), *a) for a in at(G + ATT_LAG[3], ds)])

    @_memo
    def wo_rows(nt, g):
        blk = wo_v[pl.ds(g * R, R), pl.ds(nt * L, min(L, D - nt * L))].astype(F32)
        if blk.shape[1] < L:
            blk = jnp.concatenate([blk, jnp.zeros((R, L - blk.shape[1]), F32)], axis=1)
        wo32[nt, pl.ds(g * R, R)] = blk

    @_memo
    def wo_t(nt, kt):
        def rows(g, d):
            if g >= G:
                return jnp.zeros((8, L), F32)
            wo_rows(nt, g)
            return wo32[nt, pl.ds(g * R + d, 8, stride=DH), :]
        blk = jnp.concatenate([rows(*divmod(16 * kt + j, DH)) for j in range(16)], axis=0)
        return pack(wo_s, (nt, kt), blk.astype(BF16).T)[:min(L, D - nt * L) // 2]

    wo_all = _memo(lambda kt: jnp.concatenate([wo_t(nt, kt) for nt in range(5)], axis=0))
    attn_all = _memo(lambda t: pltpu.bitcast(jnp.concatenate(
        [attn(t, g, d) for g in range(G) for d in range(0, DH, DU)], axis=0), BF16))
    proj = _memo(lambda g, t: dot([wo_all(kt)[g * R // 2:(g + 1) * R // 2] for kt in range(5)],
                                  attn_all(t)))
    x2 = _memo(lambda t: x_tile(t) + mod(2) * jnp.concatenate([proj(g, t) for g in range(G)], axis=0))
    ln2 = _memo(lambda t: layernorm(P(x2, t), 4, 3))

    def operand_units(words, idx, n):
        tok = _memo(lambda k, o: token(*words(k, o).values()))
        return [P(lambda k, o, r: pending.append(tok(k, o)[r:r + 8]), k, o, r)
                for o in _OUTER for k in idx for r in range(0, n // 2, 8)]

    h_rem = _memo(lambda t: pack(hr_s, t, ln2(t)[0]()[4 * L:]))
    h_outer = _memo(lambda b: _outer(_SB, lambda r, j: ln2(4 * b + j)[0]()[r * L:(r + 1) * L]))

    @_memo
    def h_words(b, o):
        def operand(i):
            if o not in _REM:
                return _comb(_SB[i], P(h_outer(b), o))
            low = _comb(_SB[i], lambda qi: h_outer(b)(o, qi)[:L // 2])
            high = _comb(_SB[i], lambda qi: h_outer(b)(o, qi ^ 1)[L // 2:])
            return jnp.concatenate([low, -high if i in (1, 4) else high], axis=0)
        return {i: pack(hc_s, (b, 7 * o + i), operand(i)) for i in range(7)}

    @_memo
    def up_rhs(b, o, i):
        a = h_words(b, o)
        if o not in _REM:
            return pltpu.bitcast(a[i], BF16)
        zero = jnp.zeros((L // 4, L), U32)
        rem = [h_rem(4 * b + 2 * _REM[o][1] + j) for j in range(2)]
        low = {7: zero, 8: rem[0], 9: rem[1]}[i] if i > 6 else a[i][:L // 4]
        high = ({0: zero, 5: rem[1], 6: rem[0]}[i] if i in (0, 5, 6)
                else a[{2: 3, 3: 2, 7: 0, 8: 5, 9: 6}.get(i, i)][L // 4:])
        return pltpu.bitcast(jnp.concatenate([low, high], axis=0), BF16)

    @_memo
    def w1_t(c, r, k):
        u = pltpu.bitcast(w1_v[pl.ds(k * L, min(L, D - k * L)), pl.ds((4 * c + r) * L, L)], U32)
        u = [lax.select(never, pltpu.bitcast(lane_after(recent()), U32), u[:8]), u[8:]]
        return pltpu.bitcast(jnp.concatenate(u * (1 + k // 4), axis=0), BF16).T.astype(F32)

    b1 = _memo(lambda: b1_v[...].astype(F32))
    b1_col = _memo(lambda c, r: _cols(GA * b1()[4 * c + r:][:1]))
    w1_outer = _memo(lambda c: _outer(_SA, P(w1_t, c)))
    low_lanes = lax.broadcasted_iota(jnp.int32, (L // 2, L), 1) < L // 2

    @_memo
    def w1_words(c, o):
        a = {i: pack(w1c_s, (c, 7 * o + i), _comb(_SA[i], P(w1_outer(c), o))) for i in range(7)}
        if o in _REM:
            rem = [pack(w1r_s, (c, 2 * o + ri), _comb(_REM[o][0], lambda ro: w1_t(c, 2 * ro + ri, 4)))
                   for ri in range(2)]
            a.update({i: lax.select(low_lanes, low, high) for i, low, high in (
                (2, a[2], a[3]), (3, a[3], a[2]), (5, a[5], rem[1]), (6, a[6], rem[0]),
                (8, rem[1], a[5]), (9, rem[0], a[6]))})
        return a

    w2_outer = _memo(lambda c: _outer(
        _SA, lambda r, k: w2t_v[pl.ds(r * R, R), pl.ds((4 * c + k) * L, L)].astype(F32)))
    w2_words = _memo(lambda c, o: {
        i: pack(w2c_s, (c, 7 * o + i), _comb(_SA[i], P(w2_outer(c), o))) for i in range(7)})

    up = _memo(lambda b, c, o, i: dot([w1_words(c, o)[0 if i == 7 else i]], up_rhs(b, o, i)))

    @_memo
    def up_inner(b, c, o, qi):
        v = _result(qi, P(up, b, c, o))
        return v + (up(b, c, o, 7) + up(b, c, o, 10 - qi)) if o in _REM and qi in (1, 2) else v

    def hidden(b, c, r, j):
        w = _result(r // 2 * 2 + j // 2, lambda o: up_inner(b, c, o, r % 2 * 2 + j % 2)) + b1_col(c, r)
        return w + w * jnp.tanh(w * (_C / GA + w * w))

    g_outer = _memo(lambda b, c: _outer(_SB, P(hidden, b, c)))
    g_token = _memo(lambda b, c, qi: token(*[g_outer(b, c)(o, qi) for o in (0, 2, 3, 5, 6)]))
    chunks = [range(sum(SPANS[:k]), sum(SPANS[:k + 1])) for k in range(len(SPANS))]

    @_memo
    def down(b, k, o, i):
        rhs = jnp.concatenate([_comb(_SB[i], P(g_outer(b, c), o)) for c in chunks[k]], axis=0)
        y = dot([w2_words(c, o)[i] for c in chunks[k]], rhs.astype(BF16))
        if k == 0:
            return y
        acc = down(b, k - 1, o, i)
        return jnp.concatenate([y[:16] + acc[:16], y[16:] + acc[16:]], axis=0)

    b2_col = _memo(lambda: column(b2_v[...].astype(F32).reshape(1, D)))
    gate = _memo(lambda: (0.5 / GA * mod(5), mod(5) * b2_col()))
    down_inner = _memo(lambda b, o, qi: _result(qi, P(down, b, len(SPANS) - 1, o)))

    @_memo
    def out_block(b, qo, qi):
        r, j = _rc(qo, qi)
        rs = slice(r * R, (r + 1) * R)
        y = _result(qo, lambda o: down_inner(b, o, qi))
        return pack(out_v, 4 * (4 * b + j) + r, (x2(4 * b + j)[rs] + gate()[1][rs]) + gate()[0][rs] * y)

    out_token = _memo(lambda b, qi: token(*[out_block(b, qo, qi) for qo in range(4)]))

    def write_back(b, qo):
        for qi in range(4):
            out_block(b, qo, qi)
        for qi in range(4):
            r, j = _rc(qo, qi)
            pltpu.make_async_copy(out_v.at[4 * (4 * b + j) + r],
                                  out_hbm.at[pl.ds(r * R, R), pl.ds((4 * b + j) * L, L)], out_sem).start()

    order = [(p, t) for p in range(2) for t in range(X0)] + [(2, 0), (0, X0), (2, 1)]
    for t in range(X0, NT + 2):
        order += [e for e in ((0, t + 1), (1, t), (2, t - 2)) if e[1] < NT]
        order += [(3, t - PROJ_FROM)] * (0 <= t - PROJ_FROM < PROJ_EARLY)
    when = {e: k / 4 for k, e in enumerate(order)}
    att = []
    for t in range(NT + 3):
        ready = [when[1, min(t, NT - 1)] + 0.3499, when[0, min(t + 1, NT - 1)] + 0.3499]
        ready += [when[2, min(t - 2, NT - 1)] + 0.075] if t >= 2 else []
        att.append(max(ready + [a + ATT_STEP[(t > 2) + (t > NT)] for a in att[-1:]]))
    att.append(att[-1] + 0.2)
    for t in range(PROJ_EARLY, NT):
        when[3, t] = max(max(when.values()) + 0.25, att[t + 4])
    arrive = (when[0, 2], when[1, 2], T_WAVE3, T_WAVE4)
    assert when[0, X1 - 1] >= T_WAVE3 and all(when[3, t] >= att[t + 4] for t in range(NT))
    items = [(t, P(wait, ds)) for t, ds in zip(arrive, waves)]
    items += [(t, P(start, ds)) for t, ds in zip((0,) + arrive[1:], waves[1:])]

    def spread(fs, t0, t1, vector=True):
        for j, f in enumerate(fs):
            t = t0 + (t1 - t0) * (j + 0.5) / len(fs)
            for tb in arrive:
                if vector and tb <= t < min(tb + 0.5, t1):
                    t = tb + 0.3 * min(0.5, t1 - tb) + 0.7 * (t - tb)
            items.append((t, f))

    for (p, t), s in when.items():
        spread([P(qkv, p, g, t) if p < 3 else P(proj, g, t) for g in range(G)],
               s, s + (0.25 if s < T_MLP else 1e-3), False)
    stats_end, h2_end = [T_WAVE3 + 1 + 0.4 * T_MOD], [T_WAVE3 + 1 + T_MOD]
    for t in range(NT):
        if t:
            spread(ln1(t)[1] + [P(lambda t, r: anchor(h1(t)[r:r + 24]), t, r) for r in range(0, D // 2, 24)],
                   when[1, 3] if t == X0 else when[0, t - 1], when[0, t])
        stats_end.append(max(when[3, t] + 0.3, stats_end[-1]) + T_LN)
        spread(ln2(t)[1], stats_end[-1] - T_LN, stats_end[-1])
        h2_end.append(max(stats_end[-1], h2_end[-1]) + T_LN)
        spread([P(lambda t, r: anchor(ln2(t)[0]()[r:r + 32]), t, r) for r in range(0, 4 * L, 32)]
               + [P(lambda t: anchor(h_rem(t)), t)], h2_end[-1] - T_LN, h2_end[-1])
    for p in (1, 2):
        spread([P(lambda *a: anchor(wqkv_t(*a)), p * G + g, kt) for g in range(G) for kt in range(5)],
               arrive[p - 1], when[p, 0])
    for t in range(NT + 3):
        spread(sum([attn_units(t * G + g) for g in range(G)], []), att[t], att[t + 1])
    spread([P(lambda *a: anchor(wo_t(*a)), nt, kt) for nt in range(5) for kt in range(5)],
           T_WAVE3, when[3, 0])
    for tiles, t0, t1 in ((range(9, 23), T_WAVE3 + 0.5, T_WAVE3 + 0.5 + T_MOD),
                          (range(23, 27), T_MLP + 17, T_MLP + 21)):
        spread(sum([mod_sum(t)[1] + [P(anchor_row, mod_sum(t)[0])] for t in tiles], []), t0, t1)
        spread([P(lambda t: anchor(mod_tile(t)), t) for t in tiles], t0 + 0.4, t1 + 0.4)
    spread([lambda: anchor(b2_col())], T_MLP + 21, T_MLP + 22)

    jobs = [(b, k) for k in range(len(SPANS)) for b in range(NB)]
    up_at = {bc: T_MLP + s for s, bc in enumerate((b, c) for b, k in jobs for c in chunks[k])}
    down_at = [up_at[b, chunks[k][-1]] + 2 for b, k in jobs]
    down_at.append(down_at[-1] + SPANS[-1])
    for n in range(len(jobs) - 2, 0, -1):
        gap = down_at[n + 1] - down_at[n - 1] - SPANS[jobs[n][1]] - SPANS[jobs[n - 1][1]]
        down_at[n] = max(down_at[n], down_at[n + 1] - SPANS[jobs[n][1]] - gap / 2.4)

    late = 0.7
    prep = [(up_at[b, 0] + late, h2_end[4 * b + 4], [], operand_units(h_words, [b], L)) for b in range(NB)]
    for k, cs in enumerate(chunks):
        for c in cs:
            xpose = [P(lambda c, r, n: anchor(w1_t(c, r, n)[:8] if n < 5 else b1_col(c, r)), c, r, n)
                     for r in range(4) for n in range(6)]
            prep.append((up_at[0, c] + late, T_WAVE4 + 1, xpose, operand_units(w1_words, [c], L)))
        units = operand_units(w2_words, cs, R)
        prep += [(down_at[NB * k] + j + late, T_WAVE4, [], units[j * len(units) // len(cs):][:len(units) // len(cs)])
                 for j in range(len(cs))]
    prep.sort(key=lambda e: e[:2])
    now, step = T_PREP, 1.0
    while prep:
        now = max(now, prep[0][1])
        last, step = step, min((e[0] - now) / (j + 1) for j, e in enumerate(prep))
        _, _, xpose, units = prep.pop(0)
        spread(xpose, now - min(last, 1.0), now)
        spread(units, now, now + step)
        now += step

    def last_down(n):
        down(*jobs[-1], *_DOWN[n])
        for qo, done in _DONE.items():
            if n == done + 2:
                tok = token(*[out_block(NB - 1, qo, qi) for qi in range(4)])
                pending.extend(tok[r:r + 8] for r in range(0, R // 2, 8))
            if n == min(done + 4, len(_DOWN) - 1):
                write_back(NB - 1, qo)

    def rounds(fs, n):
        return [P(lambda fs: [f() for f in fs], fs[j:j + n]) for j in range(0, len(fs), n)]

    spread(rounds([P(up, b, c, o, i) for b, c in up_at for o, i in _UP], 4),
           T_MLP - 0.1, T_MLP + len(up_at) - 0.1, False)
    for n, (b, k) in enumerate(jobs):
        fs = [P(last_down, m) if (b, k) == jobs[-1] else P(down, b, k, *oi) for m, oi in enumerate(_DOWN)]
        spread(rounds(fs, 4 // SPANS[k]), down_at[n], down_at[n + 1], False)
    for (b, c), s in up_at.items():
        spread([P(lambda b, c, qi, r: pending.append(g_token(b, c, qi)[r:r + 8]), b, c, qi, r)
                for r in range(0, L, 8) for qi in (0, 2, 3, 1)], s + 1, s + 2)
    for b in range(NB - 1):
        s = down_at[b - NB]
        spread([P(lambda b, qi, r: pending.append(out_token(b, qi)[r:r + 8]), b, qi, r)
                for r in range(0, R // 2, 8) for qi in range(4)], s + 0.1, s + 3)
        spread([P(write_back, b, qo) for qo in range(4)], s + 3.2, s + 3.5, False)

    d_m0.wait()
    mod(0)
    d_m1.wait()
    mod(1)
    d_wq.wait()
    start(waves[0])
    for g in range(G):
        for kt in range(5):
            wqkv_t(g, kt)
    d_x0.wait()
    for _, f in sorted(items, key=lambda e: e[0]):
        f()
    pltpu.make_async_copy(out_v, out_v, out_sem).wait()


@jax.jit
def pallas_adaLN_cond__sliding_local_dilated__dense_activation_gelu__prompt_kernel(
    A_x: jax.Array,
    A_wqkv: jax.Array,
    A_wo: jax.Array,
    B_x: jax.Array,
    B_w1: jax.Array,
    B_b1: jax.Array,
    B_w2: jax.Array,
    B_b2: jax.Array,
    c: jax.Array,
    w_mod: jax.Array,
):
    del B_x

    def pieces(cuts):
        return [pltpu.VMEM((D, b - a), BF16) for a, b in zip(cuts, cuts[1:])]

    scratch = [
        pieces(_X_CUTS), pieces(_QKV_CUTS), pieces(_MOD_CUTS),
        pltpu.VMEM((D, D), BF16),
        pltpu.VMEM((D, F), BF16),
        pltpu.VMEM((F // L, L), BF16),
        pltpu.VMEM((D, F), BF16),
        pltpu.VMEM((D,), BF16),
        pltpu.VMEM((1, D), BF16),
        pltpu.VMEM((5, 3 * D, L), F32),
        pltpu.VMEM((5, D, L), F32),
        pltpu.VMEM((3 * G, 5, R, L), BF16),
        pltpu.VMEM((5, 5, L, L), BF16),
        pltpu.VMEM((NT, D, L), BF16),
        pltpu.VMEM((NT, G * DH // DU, DU * 8, L), BF16),
        pltpu.VMEM((NB, 49, L, L), BF16),
        pltpu.VMEM((NT, L // 2, L), BF16),
        pltpu.VMEM((NC, 49, L, L), BF16),
        pltpu.VMEM((NC, 14, L, L), BF16),
        pltpu.VMEM((NC, 49, R, L), BF16),
        pltpu.VMEM((4 * NT, R, L), BF16),
        pltpu.SemaphoreType.DMA((17,)),
        pltpu.SemaphoreType.DMA(()),
    ]
    hbm = pl.BlockSpec(memory_space=pl.ANY)
    out_t = pl.pallas_call(
        _kernel,
        out_shape=jax.ShapeDtypeStruct((D, S), BF16),
        in_specs=[hbm] * 9,
        out_specs=hbm,
        scratch_shapes=scratch,
        compiler_params=pltpu.CompilerParams(vmem_limit_bytes=126 * 2**20),
    )(A_x[0].T, A_wqkv, A_wo, B_w1, B_b1.reshape(F // L, L), B_w2.T, B_b2, c, w_mod)
    return out_t.T[None]
```
